```python
import os as _os
_os.environ.setdefault("JAX_PLATFORMS", "cpu")
import jax
import jax.numpy as jnp

def _softmax(x, axis=-1):
    return jax.nn.softmax(x, axis=axis)
def _gelu(x):
    return jax.nn.gelu(x, approximate=True)
def _silu(x):
    return jax.nn.silu(x)
def _sigmoid(x):
    return jax.nn.sigmoid(x)
def _layernorm(x, axis=-1, eps=1e-5):
    m = jnp.mean(x, axis=axis, keepdims=True)
    v = jnp.var(x, axis=axis, keepdims=True)
    return (x - m) / jnp.sqrt(v + eps)
def _scatter_add(tgt, idx, src, axis=0):
    return tgt.at[idx].add(src)
def _segment_sum(src, seg, n):
    return jax.ops.segment_sum(src, seg, n)
class _Rng:
    def __init__(self, key):
        self._k = key
    def _next(self):
        self._k, sub = jax.random.split(self._k)
        return sub
    def normal(self, shape):
        return jax.random.normal(self._next(), shape, dtype=jnp.bfloat16)
    def randint(self, lo, hi, shape):
        return jax.random.randint(self._next(), shape, lo, hi, dtype=jnp.int32)
    def uniform(self, shape, lo=0.0, hi=1.0):
        return jax.random.uniform(self._next(), shape, jnp.bfloat16, lo, hi)
    def permutation(self, n):
        return jax.random.permutation(self._next(), n)


kernel_name = 'gated_mix__spectral_gfnet__dense_activation_silu__prompt'

def setup_inputs():
    _rng = _Rng(jax.random.key(int.from_bytes(__import__("os").urandom(4), "little")))
    _w = (lambda a: (lambda t: t.astype(jnp.bfloat16) if jnp.issubdtype(t.dtype, jnp.floating) else t)(jnp.asarray(a)))
    def _A_setup():
        B, S, D = 1, 2048, 512
        Df = D // 2 + 1
        return {
            "x": _w((lambda *s: _rng.normal(s) * 0.05)(B, S, D)),
            "w_r": _w((lambda *s: _rng.normal(s) * 0.05)(S, Df) * 0.02),
            "w_i": _w((lambda *s: _rng.normal(s) * 0.05)(S, Df) * 0.02),
        }
    _A_in = _A_setup()

    def _B_setup():
        B, S, D, F = 1, 2048, 512, 1376
        return {
            "x": _w((lambda *s: _rng.normal(s) * 0.05)(B, S, D)),
            "w1": _w((lambda *s: _rng.normal(s) * 0.05)(D, F) * (D ** -0.5)),
            "w2": _w((lambda *s: _rng.normal(s) * 0.05)(F, D) * (F ** -0.5)),
        }
    _B_in = _B_setup()

    return {
        "A_x": _A_in["x"],
        "A_w_r": _A_in["w_r"],
        "A_w_i": _A_in["w_i"],
        "B_x": _B_in["x"],
        "B_w1": _B_in["w1"],
        "B_w2": _B_in["w2"],
        "gate_w": _w((lambda *s: _rng.normal(s) * 0.05)(512) * 16.0),
    }

def reference(A_x, A_w_r, A_w_i, B_x, B_w1, B_w2, gate_w):
    def _A_ref(x, w_r, w_i):
        B, S, D = x.shape
        X = (lambda x, axes=(-2,-1): jnp.fft.rfft2(x.astype(jnp.float32), axes=axes))(x, axes=(-2, -1))
        W = w_r + 1j * w_i
        X = X * W
        y = (lambda x, s, axes=(-2,-1): jnp.fft.irfft2(x, s=s, axes=axes).astype(jnp.bfloat16))(X, (S, D), axes=(-2, -1))
        return y

    def _B_ref(x, w1, w2):
        h = jnp.einsum("bsd,df->bsf", x, w1)
        h = _silu(h)
        out = jnp.einsum("bsf,fd->bsd", h, w2)
        return out

    x = A_x
    g = _sigmoid((x * gate_w).sum(-1, keepdims=True))
    a = _A_ref(x, A_w_r, A_w_i)
    b = _B_ref(x, B_w1, B_w2)
    return g * a + (1 - g) * b
```

```python
import numpy as np
import jax
import jax.numpy as jnp
import jax.experimental.pallas as pl
import jax.experimental.pallas.tpu as pltpu

S, D, F = 2048, 512, 1376
TM = 256
NC = S // TM
RT = 272
f32, bf16 = jnp.float32, jnp.bfloat16
NT = (((1,), (1,)), ((), ()))


def _tables():
    pi2 = 2 * np.pi
    b = np.arange(128)[None, :]
    r = np.arange(64)[:, None]
    ph = lambda kd: pi2 * kd * b / 512.0
    g0 = np.zeros((144, 128))
    g0[0:64], g0[64:128] = np.cos(ph(4 * r)), -np.sin(ph(4 * r))
    g0[128] = np.cos(ph(256))[0]
    g2 = np.concatenate([np.cos(ph(4 * r + 2)), -np.sin(ph(4 * r + 2))], 0)
    c1, s1, c3, s3 = np.cos(ph(4 * r + 1)), np.sin(ph(4 * r + 1)), np.cos(ph(4 * r + 3)), np.sin(ph(4 * r + 3))
    g1 = np.block([[c1, s1], [c3, -s3], [-s1, c1], [-s3, -c3]])
    sc = 1.0 / (S * D)
    h0 = 2 * g0[:128].copy()
    h0[0] = 1.0
    h0[64] = g0[128]
    small = np.zeros((912, 256))
    small[0:144, :128] = g0
    small[144:272, :128] = g2
    small[272:528] = g1
    small[528:656, :128] = h0 * sc
    small[528:656, 128:] = 2 * g2 * sc
    small[656:912] = 2 * g1 * sc
    n1 = np.arange(128)[:, None]
    k1 = np.arange(128)[None, :]
    m = []
    for n2 in range(16):
        a = pi2 * (k1 * (16 * n1 + n2) % S) / S
        c, s = np.cos(a), -np.sin(a)
        m.append(np.block([[c, s], [-s, c]]))
    return small.astype(np.float32), np.stack(m).astype(np.float32)


_SMALL, _MTAB = _tables()


def _fft4(x, sg):
    (ar, ai), (br, bi), (cr, ci), (dr, di) = x
    s0r, s0i, d0r, d0i = ar + cr, ai + ci, ar - cr, ai - ci
    s1r, s1i, d1r, d1i = br + dr, bi + di, br - dr, bi - di
    if sg < 0:
        o1, o3 = (d0r + d1i, d0i - d1r), (d0r - d1i, d0i + d1r)
    else:
        o3, o1 = (d0r + d1i, d0i - d1r), (d0r - d1i, d0i + d1r)
    return [(s0r + s1r, s0i + s1i), o1, (s0r - s1r, s0i - s1i), o3]


def _tw(z, e, sg):
    e %= 16
    zr, zi = z
    if e == 0:
        return z
    if e == 4:
        return (zi, -zr) if sg < 0 else (-zi, zr)
    c, s = float(np.cos(2 * np.pi * e / 16)), float(sg * np.sin(2 * np.pi * e / 16))
    if e % 2 == 0:
        if c * s > 0:
            return ((zr - zi) * c, (zr + zi) * c)
        return ((zr + zi) * c, (zi - zr) * c)
    return (zr * c - zi * s, zr * s + zi * c)


def _fft16(x, sg):
    t = [_fft4([x[4 * a + b] for a in range(4)], sg) for b in range(4)]
    out = [None] * 16
    for p in range(4):
        o = _fft4([_tw(t[b][p], b * p, sg) for b in range(4)], sg)
        for q in range(4):
            out[p + 4 * q] = o[q]
    return out


def _kernel(x_hbm, wr_hbm, wi_hbm, w1_hbm, w2_hbm, gw_ref, sm_hbm, m_hbm, o_hbm,
            x_v, wr_v, wi_v, w1_v, w2_v, sm_v, m_v, wf, t_v, a_v, b_v, o_v, g_v, sems, osem):
    cps = [
        pltpu.make_async_copy(x_hbm.at[pl.ds(0, TM)], x_v.at[pl.ds(0, TM)], sems.at[0]),
        pltpu.make_async_copy(w1_hbm.at[pl.ds(0, 512)], w1_v.at[pl.ds(0, 512)], sems.at[1]),
        pltpu.make_async_copy(w2_hbm.at[pl.ds(0, 512)], w2_v.at[pl.ds(0, 512)], sems.at[2]),
        pltpu.make_async_copy(w1_hbm.at[pl.ds(512, F - 512)], w1_v.at[pl.ds(512, F - 512)], sems.at[3]),
        pltpu.make_async_copy(w2_hbm.at[pl.ds(512, F - 512)], w2_v.at[pl.ds(512, F - 512)], sems.at[4]),
        pltpu.make_async_copy(x_hbm.at[pl.ds(TM, S - TM)], x_v.at[pl.ds(TM, S - TM)], sems.at[5]),
        pltpu.make_async_copy(wr_hbm, wr_v, sems.at[6]),
        pltpu.make_async_copy(wi_hbm, wi_v, sems.at[7]),
        pltpu.make_async_copy(sm_hbm, sm_v, sems.at[8]),
        pltpu.make_async_copy(m_hbm, m_v, sems.at[9]),
    ]
    for c in cps:
        c.start()

    def ffn(r0, first=False):
        xx = x_v[pl.ds(r0, TM), :]
        acc = None
        for j, (f0, f1) in enumerate(((0, 512), (512, 1024), (1024, F))):
            if first and j < 2:
                cps[1 + 2 * j].wait()
            h = jax.lax.dot_general(xx, w1_v[f0:f1, :], NT, preferred_element_type=f32)
            h = (h * jax.nn.sigmoid(h)).astype(bf16)
            if first and j < 2:
                cps[2 + 2 * j].wait()
            p = jnp.dot(h, w2_v[f0:f1, :], preferred_element_type=f32)
            acc = p if acc is None else acc + p
        b_v[pl.ds(r0, TM), :] = acc
        g = jax.nn.sigmoid(jnp.sum(xx.astype(f32) * gw_ref[...].astype(f32).reshape(1, D), axis=-1, keepdims=True))
        g_v[pl.ds(r0, TM), :] = jnp.broadcast_to(g, (TM, 128))

    cps[0].wait()
    ffn(0, True)
    cps[5].wait()
    ffn(TM)
    cps[6].wait()
    cps[7].wait()
    cps[8].wait()
    for a in range(4):
        a_v[a] = x_v[:, 128 * a:128 * a + 128].astype(f32)
    for j in range(16):
        wf[0, j] = wr_v[0:256, 128 * j:128 * j + 128].astype(f32)
        wf[1, j] = wi_v[0:256, 128 * j:128 * j + 128].astype(f32)
    ffn(7 * TM)
    cps[9].wait()


    def fwd(m, c):
        halves = [[a_v[a, pl.ds(2 * m + e, 128, stride=16), :] for a in range(4)] for e in range(2)]
        for e, xv in enumerate(halves):
            n2 = 2 * m + e
            x0, x1, x2, x3 = xv
            s02, s13 = x0 + x2, x1 + x3
            y0, y2 = (s02 + s13).astype(bf16), (s02 - s13).astype(bf16)
            y1 = jnp.concatenate([x0 - x2, x3 - x1], axis=1).astype(bf16)
            p = jax.lax.dot_general(sm_v[0:144, 0:128], y0, NT, preferred_element_type=f32).astype(bf16)
            q = jax.lax.dot_general(sm_v[144:272, 0:128], y2, NT, preferred_element_type=f32).astype(bf16)
            z = jax.lax.dot_general(sm_v[272:528, :], y1, NT, preferred_element_type=f32).astype(bf16)
            yr = jnp.concatenate([p[0:64], q[0:64], z[0:128], p[128:144]], axis=0)
            yi = jnp.concatenate([p[64:128], q[64:128], z[128:256], jnp.zeros((16, 128), bf16)], axis=0)
            t_v[n2] = jnp.dot(jnp.concatenate([yr, yi], axis=1), m_v[n2], preferred_element_type=f32)
        return c

    [fwd(m, 0) for m in range(8)]

    def filt(row, wload):
        z = _fft16([(t_v[j, pl.ds(row, 8), 0:128], t_v[j, pl.ds(row, 8), 128:256]) for j in range(16)], -1)
        y = []
        for j in range(16):
            wr, wi = wload(j)
            y.append((z[j][0] * wr - z[j][1] * wi, z[j][0] * wi + z[j][1] * wr))
        y = _fft16(y, 1)
        for j in range(16):
            t_v[j, pl.ds(row, 8), 0:128] = y[j][0]
            t_v[j, pl.ds(row, 8), 128:256] = y[j][1]

    def mid(i, c):
        ffn(pl.multiple_of((2 + i) * TM, TM))
        for g in range(2):
            r = pl.multiple_of(i * 16 + g * 8, 8)
            for blk, off in enumerate((0, 2, 1, 3)):
                filt(r + 64 * blk, lambda j: tuple(
                    wf[e, j, pl.ds(4 * r + off, 8, stride=4), :] for e in range(2)))
        return c

    jax.lax.fori_loop(0, 4, mid, 0)
    filt(256, lambda j: tuple(
        jnp.broadcast_to(v[256:257, 128 * j:128 * j + 128].astype(f32), (8, 128)) for v in (wr_v, wi_v)))

    def inv(n2, c):
        t = t_v[n2]
        tr, ti = t[:, 0:128], t[:, 128:256]
        row = jax.lax.broadcasted_iota(jnp.int32, (64, 256), 0)
        nyq = jnp.broadcast_to(t[256:257], (64, 256))
        w0 = jnp.concatenate([t[0:64], jnp.where(row == 0, nyq, jnp.concatenate([ti[0:64], -tr[0:64]], 1))], 0)
        w2 = jnp.concatenate([t[64:128], jnp.concatenate([ti[64:128], -tr[64:128]], 1)], 0)
        w02 = jnp.concatenate([w0, w2], 0).astype(bf16)
        pq = jax.lax.dot_general(m_v[n2, 0:128, :], w02, NT, preferred_element_type=f32).astype(bf16)
        z = jax.lax.dot_general(m_v[n2], t[128:256].astype(bf16), NT, preferred_element_type=f32).astype(bf16)
        y0 = jnp.dot(pq[:, 0:128], sm_v[528:656, 0:128], preferred_element_type=f32)
        y2 = jnp.dot(pq[:, 128:256], sm_v[528:656, 128:256], preferred_element_type=f32)
        y1 = jnp.dot(jnp.concatenate([z[0:128], z[128:256]], 1), sm_v[656:912, :], preferred_element_type=f32)
        e, o = y0 + y2, y0 - y2
        u, v = y1[:, 0:128], y1[:, 128:256]
        for a, val in enumerate((e + u, o - v, e - u, o + v)):
            a_v[a, pl.ds(n2, 128, stride=16), :] = val
        return c

    [inv(m, 0) for m in range(16)]

    def ocopy(c):
        return pltpu.make_async_copy(o_v.at[pl.ds(c * TM, TM)], o_hbm.at[pl.ds(c * TM, TM)], osem.at[c])

    def mix(c):
        rows = pl.ds(c * TM, TM)
        g = jnp.tile(g_v[rows, :], (1, 4))
        b = b_v[rows, :]
        o_v[rows, :] = (b + g * (jnp.concatenate([a_v[a, rows, :] for a in range(4)], 1) - b)).astype(bf16)
        ocopy(c).start()

    for c in (0, 1, 2, 3, 4, 5, 7):
        mix(c)
    ffn(6 * TM)
    mix(6)
    for c in range(NC):
        ocopy(c).wait()


@jax.jit
def pallas_gated_mix__spectral_gfnet__dense_activation_silu__prompt_kernel(
    A_x: jax.Array,
    A_w_r: jax.Array,
    A_w_i: jax.Array,
    B_x: jax.Array,
    B_w1: jax.Array,
    B_w2: jax.Array,
    gate_w: jax.Array,
):
    hbm = pl.BlockSpec(memory_space=pl.ANY)
    V = pltpu.VMEM
    out = pl.pallas_call(
        _kernel,
        in_specs=[hbm] * 5 + [pl.BlockSpec(memory_space=V), hbm, hbm],
        out_specs=hbm,
        out_shape=jax.ShapeDtypeStruct((S, D), bf16),
        scratch_shapes=[
            V((S, D), bf16), V((257, S), bf16), V((257, S), bf16),
            V((F, D), bf16), V((F, D), bf16), V((912, 256), bf16), V((16, 256, 256), bf16),
            V((2, 16, 256, 128), f32), V((16, RT, 256), f32), V((4, S, 128), f32), V((S, D), f32), V((S, D), bf16), V((S, 128), f32),
            pltpu.SemaphoreType.DMA((10,)), pltpu.SemaphoreType.DMA((NC,)),
        ],
        compiler_params=pltpu.CompilerParams(vmem_limit_bytes=100 * 1024 * 1024),
    )(A_x.reshape(S, D), A_w_r.T, A_w_i.T, B_w1.T, B_w2,
      gate_w, jnp.asarray(_SMALL, bf16), jnp.asarray(_MTAB, bf16))
    return out.reshape(1, S, D)
```
